```python
import jax
import jax.numpy as jnp

def _softmax(x, axis=-1):
    return jax.nn.softmax(x, axis=axis)

def _gelu(x):
    return jax.nn.gelu(x, approximate=True)

def _silu(x):
    return jax.nn.silu(x)

def _sigmoid(x):
    return jax.nn.sigmoid(x)

def _layernorm(x, axis=-1, eps=1e-05):
    m = jnp.mean(x, axis=axis, keepdims=True)
    v = jnp.var(x, axis=axis, keepdims=True)
    return (x - m) / jnp.sqrt(v + eps)

def _scatter_add(tgt, idx, src, axis=0):
    return tgt.at[idx].add(src)

def _segment_sum(src, seg, n):
    return jax.ops.segment_sum(src, seg, n)

class _Rng:

    def __init__(self, key):
        self._k = key

    def _next(self):
        self._k, sub = jax.random.split(self._k)
        return sub

    def normal(self, shape):
        return jax.random.normal(self._next(), shape, dtype=jnp.bfloat16)

    def randint(self, lo, hi, shape):
        return jax.random.randint(self._next(), shape, lo, hi, dtype=jnp.int32)

    def uniform(self, shape, lo=0.0, hi=1.0):
        return jax.random.uniform(self._next(), shape, jnp.bfloat16, lo, hi)

    def permutation(self, n):
        return jax.random.permutation(self._next(), n)
kernel_name = 'adaLN_cond__sliding_block_cached__mixer_gmlp__decode'

def setup_inputs():
    _rng = _Rng(jax.random.key(int.from_bytes(__import__("os").urandom(4), "little")))
    _w = lambda a: (lambda t: t.astype(jnp.bfloat16) if jnp.issubdtype(t.dtype, jnp.floating) else t)(jnp.asarray(a))

    def _A_setup():
        B, Sq, D = (1, 1, 448)
        Hq, Hkv, Sk, Dh = (16, 8, 65536, 256)
        assert Hq % Hkv == 0, (Hq, Hkv)
        return {'x': _w((lambda *s: _rng.normal(s) * 0.05)(B, Sq, D)), 'k_cache': _w((lambda *s: _rng.normal(s) * 0.05)(B, Hkv, Sk, Dh)), 'v_cache': _w((lambda *s: _rng.normal(s) * 0.05)(B, Hkv, Sk, Dh)), 'wq': _w((lambda *s: _rng.normal(s) * 0.05)(D, Hq * Dh) * D ** (-0.5)), 'wo': _w((lambda *s: _rng.normal(s) * 0.05)(Hq * Dh, D) * (Hq * Dh) ** (-0.5))}
    _A_in = _A_setup()

    def _B_setup():
        B, S, D, F = (1, 1, 448, 1792)
        Fh = F // 2
        return {'x': _w((lambda *s: _rng.normal(s) * 0.05)(B, S, D)), 'w_in': _w((lambda *s: _rng.normal(s) * 0.05)(D, 2 * Fh)), 'w_sp': _w(0.01 * (lambda *s: _rng.normal(s) * 0.05)(S, S)), 'b_sp': _w(1.0 + 0.01 * (lambda *s: _rng.normal(s) * 0.05)(S)), 'w_out': _w((lambda *s: _rng.normal(s) * 0.05)(Fh, D))}
    _B_in = _B_setup()
    return {'A_x': _A_in['x'], 'A_k_cache': _A_in['k_cache'], 'A_v_cache': _A_in['v_cache'], 'A_wq': _A_in['wq'], 'A_wo': _A_in['wo'], 'B_x': _B_in['x'], 'B_w_in': _B_in['w_in'], 'B_w_sp': _B_in['w_sp'], 'B_b_sp': _B_in['b_sp'], 'B_w_out': _B_in['w_out'], 'c': _w((lambda *s: _rng.normal(s) * 0.05)(1, 448)), 'w_mod': _w((lambda *s: _rng.normal(s) * 0.05)(448, 6 * 448) * 448 ** (-0.5))}

def reference(A_x, A_k_cache, A_v_cache, A_wq, A_wo, B_x, B_w_in, B_w_sp, B_b_sp, B_w_out, c, w_mod):

    def _A_ref(x, k_cache, v_cache, wq, wo):
        B, Sq, D = x.shape
        Hq, Dh = (16, 256)
        Hkv, Sk = (k_cache.shape[1], k_cache.shape[2])
        W = min(4096, max(256, Sk // 4))
        rep = Hq // Hkv
        q = (lambda x, *d: x.transpose(*d))((x @ wq).reshape(B, Sq, Hq, Dh), 0, 2, 1, 3)
        k = jnp.repeat(k_cache[:, :, Sk - W:, :], rep, axis=1)
        v = jnp.repeat(v_cache[:, :, Sk - W:, :], rep, axis=1)
        scores = jnp.einsum('bhqd,bhkd->bhqk', q, k) * Dh ** (-0.5)
        p = _softmax(scores, axis=-1)
        o = jnp.einsum('bhqk,bhkd->bhqd', p, v)
        return (lambda x, *d: x.transpose(*d))(o, 0, 2, 1, 3).reshape(B, Sq, Hq * Dh) @ wo

    def _B_ref(x, w_in, w_sp, b_sp, w_out):
        B, S, D = x.shape
        F = w_in.shape[-1]
        Fh = F // 2
        z = _gelu(jnp.einsum('bsd,df->bsf', x, w_in))
        z1 = z[..., :Fh].copy()
        z2 = _layernorm(z[..., Fh:], axis=-1)
        g = jnp.einsum('ts,bsf->btf', w_sp, z2) + b_sp[None, :, None]
        return jnp.einsum('bsf,fd->bsd', z1 * g, w_out)
    x = A_x
    mod = (_silu(c) @ w_mod).reshape(c.shape[0], 6, 1, -1)
    sa, ca, ga, sb, cb, gb = (mod[:, 0].copy(), mod[:, 1].copy(), mod[:, 2].copy(), mod[:, 3].copy(), mod[:, 4].copy(), mod[:, 5].copy())
    h = _layernorm(x, axis=-1) * (1 + ca) + sa
    x = x + ga * _A_ref(h, A_k_cache, A_v_cache, A_wq, A_wo)
    h = _layernorm(x, axis=-1) * (1 + cb) + sb
    x = x + gb * _B_ref(h, B_w_in, B_w_sp, B_b_sp, B_w_out)
    return x
```

```python
import jax
import jax.numpy as jnp
from jax import lax
import jax.experimental.pallas as pl
import jax.experimental.pallas.tpu as pltpu

_NT = (((1,), (1,)), ((), ()))
_NN = (((1,), (0,)), ((), ()))
_EPS = 1e-05
_ROWS = 8


def _dot(a, b, dims):
    return lax.dot_general(a, b, dims, preferred_element_type=jnp.float32)


def _ln(x):
    m = jnp.mean(x, axis=-1, keepdims=True)
    d = x - m
    v = jnp.mean(d * d, axis=-1, keepdims=True)
    return d * lax.rsqrt(v + _EPS)


def _row_chunks(n, size):
    out, s = [], 0
    while s < n:
        out.append((s, min(size, n - s)))
        s += size
    return out


@jax.jit
def pallas_adaLN_cond__sliding_block_cached__mixer_gmlp__decode_kernel(
    A_x: jax.Array,
    A_k_cache: jax.Array,
    A_v_cache: jax.Array,
    A_wq: jax.Array,
    A_wo: jax.Array,
    B_x: jax.Array,
    B_w_in: jax.Array,
    B_w_sp: jax.Array,
    B_b_sp: jax.Array,
    B_w_out: jax.Array,
    c: jax.Array,
    w_mod: jax.Array,
):
    del B_x
    B, Sq, D = A_x.shape
    assert B == 1 and Sq == 1
    Hq, Dh = 16, 256
    Hkv, Sk = A_k_cache.shape[1], A_k_cache.shape[2]
    W = min(4096, max(256, Sk // 4))
    rep = Hq // Hkv
    assert rep == 2
    F = B_w_in.shape[-1]
    Fh = F // 2
    scale = Dh ** (-0.5)
    bf16, f32 = jnp.bfloat16, jnp.float32

    wo_chunks = _row_chunks(D, 128)
    win_chunks = _row_chunks(D, 128)
    wout_chunks = _row_chunks(D, 128)

    def kernel(x_hbm, k_hbm, v_hbm, wq_hbm, wot_hbm, win_hbm, wsp_hbm, bsp_hbm,
               woutt_hbm, c_hbm, wmod_hbm,
               o_ref,
               x_v, c_v, wsp_v, bsp_v, wmod_v, wq_v, k_v, v_v, wot_v, win_v, woutt_v,
               q_s, o_s, sems):
        sem_small = sems.at[pl.ds(0, 4)]
        sem_w = sems.at[pl.ds(4, 2)]
        sem_k = sems.at[pl.ds(6, Hkv)]
        sem_v = sems.at[pl.ds(6 + Hkv, Hkv)]
        o0 = 6 + 2 * Hkv
        sem_wo = sems.at[pl.ds(o0, len(wo_chunks))]
        o0 += len(wo_chunks)
        sem_win = sems.at[pl.ds(o0, len(win_chunks))]
        o0 += len(win_chunks)
        sem_wout = sems.at[pl.ds(o0, len(wout_chunks))]

        def k_copy(h):
            return pltpu.make_async_copy(
                k_hbm.at[0, h, pl.ds(Sk - W, W), :], k_v.at[h], sem_k.at[h])

        def v_copy(h):
            return pltpu.make_async_copy(
                v_hbm.at[0, h, pl.ds(Sk - W, W), :], v_v.at[h], sem_v.at[h])

        def rows_copy(src, dst, sem, i, chunk):
            s, n = chunk
            return pltpu.make_async_copy(
                src.at[pl.ds(s, n), :], dst.at[pl.ds(s, n), :], sem.at[i])

        wmod_cp = pltpu.make_async_copy(wmod_hbm, wmod_v, sem_w.at[0])
        wq_cp = pltpu.make_async_copy(wq_hbm, wq_v, sem_w.at[1])
        small = [
            pltpu.make_async_copy(c_hbm, c_v, sem_small.at[0]),
            pltpu.make_async_copy(x_hbm, x_v, sem_small.at[1]),
            pltpu.make_async_copy(wsp_hbm, wsp_v, sem_small.at[2]),
            pltpu.make_async_copy(bsp_hbm, bsp_v, sem_small.at[3]),
        ]
        wo_cps = [rows_copy(wot_hbm, wot_v, sem_wo, i, ch) for i, ch in enumerate(wo_chunks)]
        win_cps = [rows_copy(win_hbm, win_v, sem_win, i, ch) for i, ch in enumerate(win_chunks)]
        wout_cps = [rows_copy(woutt_hbm, woutt_v, sem_wout, i, ch) for i, ch in enumerate(wout_chunks)]

        wmod_cp.start()
        for cp in small:
            cp.start()
        wq_cp.start()
        for h in range(Hkv):
            k_copy(h).start()
            v_copy(h).start()
        for cp in wo_cps + win_cps + wout_cps:
            cp.start()

        for cp in small:
            cp.wait()
        x = x_v[0].astype(f32)
        cc = c_v[...].astype(f32)
        sc = cc * jax.nn.sigmoid(cc)
        sc8 = jnp.broadcast_to(sc.astype(bf16), (_ROWS, D))
        ln_x = _ln(x)

        wmod_cp.wait()
        mod = _dot(sc8, wmod_v[...], _NN)
        sa, ca, ga, sb, cb, gb = (mod[:, i * D:(i + 1) * D] for i in range(6))
        h1 = (ln_x * (1.0 + ca) + sa).astype(bf16)

        wq_cp.wait()
        q = _dot(h1, wq_v[...], _NN)
        q = (q.astype(bf16).astype(f32) * scale)
        row = lax.broadcasted_iota(jnp.int32, (_ROWS, Dh), 0)
        for g in range(Hkv):
            qa = q[:, (2 * g) * Dh:(2 * g + 1) * Dh]
            qb = q[:, (2 * g + 1) * Dh:(2 * g + 2) * Dh]
            q_s[g] = jnp.where(row == 0, qa, qb)

        def head_body(g, carry):
            k_copy(g).wait()
            qg = q_s[g].astype(bf16)
            s = _dot(qg, k_v[g], _NT)
            m = jnp.max(s, axis=-1, keepdims=True)
            p = jnp.exp(s - m)
            l = jnp.sum(p, axis=-1, keepdims=True)
            v_copy(g).wait()
            o = _dot(p.astype(bf16), v_v[g], _NN)
            o = o / l
            o_s[g] = o
            return carry

        lax.fori_loop(0, Hkv, head_body, 0)

        parts = []
        for g in range(Hkv):
            og = o_s[g]
            parts.append(jnp.where(row == 0, og, 0.0))
            parts.append(jnp.where(row == 1, og, 0.0))
        o_cat = jnp.concatenate(parts, axis=1).astype(bf16)
        attn_parts = []
        for cp, (s0, n) in zip(wo_cps, wo_chunks):
            cp.wait()
            attn_parts.append(_dot(o_cat, wot_v[pl.ds(s0, n), :], _NT))
        attn = jnp.concatenate(attn_parts, axis=1)
        attn = jnp.sum(attn, axis=0, keepdims=True)

        x1 = x + ga * attn
        h2 = (_ln(x1) * (1.0 + cb) + sb).astype(bf16)
        z = None
        for cp, (s0, n) in zip(win_cps, win_chunks):
            cp.wait()
            part = _dot(h2[:, s0:s0 + n], win_v[pl.ds(s0, n), :], _NN)
            z = part if z is None else z + part
        z = jax.nn.gelu(z, approximate=True)
        z1 = z[:, :Fh]
        z2 = _ln(z[:, Fh:])
        gate = wsp_v[...].astype(f32) * z2 + bsp_v[...].astype(f32)
        u = (z1 * gate).astype(bf16)
        y_parts = []
        for cp, (s0, n) in zip(wout_cps, wout_chunks):
            cp.wait()
            y_parts.append(_dot(u, woutt_v[pl.ds(s0, n), :], _NT))
        y = jnp.concatenate(y_parts, axis=1)
        out = x1 + gb * y
        o_ref[0] = out[0:1, :].astype(o_ref.dtype)

    any_spec = pl.BlockSpec(memory_space=pl.ANY)
    return pl.pallas_call(
        kernel,
        in_specs=[any_spec] * 11,
        out_specs=pl.BlockSpec(memory_space=pltpu.VMEM),
        out_shape=jax.ShapeDtypeStruct((B, Sq, D), A_x.dtype),
        scratch_shapes=[
            pltpu.VMEM((1, 1, D), bf16),
            pltpu.VMEM((1, D), bf16),
            pltpu.VMEM((1, 1), bf16),
            pltpu.VMEM((1, 1), bf16),
            pltpu.VMEM((D, 6 * D), bf16),
            pltpu.VMEM((D, Hq * Dh), bf16),
            pltpu.VMEM((Hkv, W, Dh), bf16),
            pltpu.VMEM((Hkv, W, Dh), bf16),
            pltpu.VMEM((D, Hq * Dh), bf16),
            pltpu.VMEM((D, F), bf16),
            pltpu.VMEM((D, Fh), bf16),
            pltpu.VMEM((Hkv, _ROWS, Dh), f32),
            pltpu.VMEM((Hkv, _ROWS, Dh), f32),
            pltpu.SemaphoreType.DMA(
                (6 + 2 * Hkv + len(wo_chunks) + len(win_chunks) + len(wout_chunks),)),
        ],
        compiler_params=pltpu.CompilerParams(vmem_limit_bytes=96 * 1024 * 1024),
    )(A_x, A_k_cache, A_v_cache, A_wq, A_wo.T, B_w_in, B_w_sp, B_b_sp.reshape(1, 1),
      B_w_out.T, c, w_mod)
```

```python
import jax
import jax.numpy as jnp
from jax import lax
import jax.experimental.pallas as pl
import jax.experimental.pallas.tpu as pltpu

_NT = (((1,), (1,)), ((), ()))
_NN = (((1,), (0,)), ((), ()))
_EPS = 1e-05
_ROWS = 8

CFG = dict(
    piece=64,
    G=4,
    sub=2,
    per=4,
    stagger=2,
    w_streams=4,
    win_streams=2,
    lag=26,
    pre=28,
    cap=60,
    wout_rows=8,
    wout_groups=(256, 128, 64),
    gb_rows=32,
    win_split=[(0, 256), (256, 192)],
    scopes=False,
)


def _dot(a, b, dims):
    return lax.dot_general(a, b, dims, preferred_element_type=jnp.float32)


def _ln(x):
    m = jnp.mean(x, axis=-1, keepdims=True)
    d = x - m
    v = jnp.mean(d * d, axis=-1, keepdims=True)
    return d * lax.rsqrt(v + _EPS)


def _round_robin(streams):
    out = []
    for j in range(max(len(s) for s in streams)):
        for s in streams:
            if j < len(s):
                out.append(s[j])
    return out


def _split(items, n):
    m = len(items)
    return [items[i * m // n:(i + 1) * m // n] for i in range(n)]


def _fold_lanes(x, op):
    parts = [x[:, i:i + 128] for i in range(0, x.shape[1], 128)]
    while len(parts) > 1:
        parts = [op(parts[i], parts[i + 1]) for i in range(0, len(parts) - 1, 2)] + (
            [parts[-1]] if len(parts) % 2 else [])
    return parts[0]


def make(cfg):
  class _Null:
    def __enter__(self): return self
    def __exit__(self, *a): return False
  def scope(name):
    return jax.named_scope(name) if cfg['scopes'] else _Null()

  def fn(
    A_x: jax.Array,
    A_k_cache: jax.Array,
    A_v_cache: jax.Array,
    A_wq: jax.Array,
    A_wo: jax.Array,
    B_x: jax.Array,
    B_w_in: jax.Array,
    B_w_sp: jax.Array,
    B_b_sp: jax.Array,
    B_w_out: jax.Array,
    c: jax.Array,
    w_mod: jax.Array,
  ):
    del B_x
    B, Sq, D = A_x.shape
    assert B == 1 and Sq == 1
    Hq, Dh = 16, 256
    Hkv, Sk = A_k_cache.shape[1], A_k_cache.shape[2]
    W = min(4096, max(256, Sk // 4))
    rep = Hq // Hkv
    assert rep == 2
    F = B_w_in.shape[-1]
    Fh = F // 2
    HD = Hq * Dh
    scale = Dh ** (-0.5)
    bf16, f32 = jnp.bfloat16, jnp.float32

    R, G, SUB, PER = cfg['piece'], cfg['G'], cfg['sub'], cfg['per']
    NGRP = Hkv // G
    SROWS = SUB * PER * R
    NSL = W // SROWS
    NPS = W // (SUB * R)
    assert NSL * SROWS == W and NGRP * G == Hkv
    MOD_EARLY = (5 * D + 127) // 128 * 128
    MOD_LATE = 6 * D - MOD_EARLY
    win_groups = [(0, D // 2), (D // 2, D - D // 2)] if not cfg.get('win_split') else cfg['win_split']
    wout_groups, r0 = [], 0
    for n in cfg['wout_groups']:
        wout_groups.append((r0, n))
        r0 += n
    assert r0 == D

    def kernel(x_hbm, k_hbm, v_hbm, wq_hbm, wot_hbm, win_hbm, wsp_hbm, bsp_hbm,
               woutt_hbm, c_hbm, wmod_hbm,
               o_ref,
               x_v, c_v, wsp_v, bsp_v, wmod_v, gbw_v, wq_v, k_v, v_v, wot_v, win_v, woutt_v,
               mod_s, s_s):
      groups = {}
      need = []

      def group(name, dst):
          groups[name] = (len(groups) + 4, dst)
          return name

      def w_pieces(name, src, dst, r0, nrows, rows, c0, ncols, cols, dc0=None):
          dc0 = c0 if dc0 is None else dc0
          return [(name, src.at[pl.ds(r, rows), pl.ds(c0 + cc, cols)],
                   dst.at[pl.ds(r, rows), pl.ds(dc0 + cc, cols)])
                  for r in range(r0, r0 + nrows, rows) for cc in range(0, ncols, cols)]

      ws = cfg['w_streams']
      need += _round_robin(_split(w_pieces(
          group('wmod', wmod_v), wmod_hbm, wmod_v, 0, D, 8, 0, MOD_EARLY, MOD_EARLY), ws))
      need += _round_robin(_split(w_pieces(
          group('wq', wq_v), wq_hbm, wq_v, 0, D, 8, 0, HD, HD // 2), ws))
      need += _round_robin(_split(w_pieces(
          group('wo', wot_v), wot_hbm, wot_v, 0, D, 8, 0, HD, HD // 2), ws))
      for g in range(NGRP):
          for t, hbm, vm in (('k', k_hbm, k_v), ('v', v_hbm, v_v)):
              for j in range(NSL):
                  name = group((t, g, j), vm.at[g * NSL + j])
                  for cidx in range(PER):
                      for u in range(SUB):
                          for hh in range(G):
                              pos = (j * PER + cidx + cfg['stagger'] * (u * G + hh)) % NPS
                              row = Sk - W + (u * NPS + pos) * R
                              need.append((
                                  name,
                                  hbm.at[0, g * G + hh, pl.ds(row, R), :],
                                  vm.at[g * NSL + j, hh, pl.ds((u * PER + cidx) * R, R), :]))
      for i, (r0, n) in enumerate(win_groups):
          need += _round_robin(_split(w_pieces(
              group(('win', i), win_v.at[pl.ds(r0, n), :]), win_hbm, win_v, r0, n, 8, 0, F, F),
              cfg['win_streams']))
      need += _round_robin(_split(w_pieces(
          group('gb', gbw_v), wmod_hbm, gbw_v, 0, D, cfg['gb_rows'], MOD_EARLY, MOD_LATE,
          MOD_LATE, 0), 2))
      for i, (r0, n) in enumerate(wout_groups):
          need += _round_robin(_split(w_pieces(
              group(('wout', i), woutt_v.at[pl.ds(r0, n), :]), woutt_hbm, woutt_v, r0, n,
              cfg['wout_rows'], 0, Fh, Fh), 2))

      lag = cfg['lag']
      n_hi = (len(need) - lag) // 2
      lo = need[0:2 * n_hi:2] + need[2 * n_hi:]
      hi = need[1:2 * n_hi:2]
      plan = [(e, 1) for e in lo[:lag]]
      for i in range(len(lo) - lag):
          if i < n_hi:
              plan.append((hi[i], 0))
          plan.append((lo[lag + i], 1))
      last = {}
      for i, (e, _) in enumerate(plan):
          last[e[0]] = i

      def body(sems):
        issued = [0]

        def issue_upto(n):
            n = min(n, len(plan))
            for (name, src, dst), prio in plan[issued[0]:n]:
                pltpu.make_async_copy(src, dst, sems.at[groups[name][0]]).start(priority=prio)
            issued[0] = max(issued[0], n)

        def wait(name):
            tag = "_".join(map(str, name)) if isinstance(name, tuple) else name
            with scope("pre_" + tag):
                issue_upto(last[name] + 1 + cfg['pre'])
            slot, dst = groups[name]
            with scope("wait_" + tag):
                pltpu.make_async_copy(dst, dst, sems.at[slot]).wait()
            with scope("post_" + tag):
                issue_upto(last[name] + 1 + cfg['cap'])

        small = [
            pltpu.make_async_copy(c_hbm, c_v, sems.at[0]),
            pltpu.make_async_copy(x_hbm, x_v, sems.at[1]),
            pltpu.make_async_copy(wsp_hbm, wsp_v, sems.at[2]),
            pltpu.make_async_copy(bsp_hbm, bsp_v, sems.at[3]),
        ]
        issue_upto(4)
        for cp in small:
            cp.start()
        issue_upto(lag + 50)
        for cp in small:
            cp.wait()
        x = jnp.broadcast_to(x_v[0].astype(f32), (_ROWS, D))
        cc = jnp.broadcast_to(c_v[...].astype(f32), (_ROWS, D))
        sc = (cc * jax.nn.sigmoid(cc)).astype(bf16)
        ln_x = _ln(x)

        wait('wmod')
        mod = _dot(sc, wmod_v[...], _NN)
        for i in range(5):
            mod_s[i] = mod[:, i * D:(i + 1) * D]
        gb_lo = mod[:, 5 * D:]
        h1 = (ln_x * (1.0 + mod_s[1]) + mod_s[0]).astype(bf16)

        wait('wq')
        q = _dot(h1, wq_v[...], _NN)
        q = q.astype(bf16).astype(f32) * scale
        row = lax.broadcasted_iota(jnp.int32, (_ROWS, Dh), 0)
        qh = [jnp.where(row == 0, q[:, (2 * h) * Dh:(2 * h + 1) * Dh],
                        q[:, (2 * h + 1) * Dh:(2 * h + 2) * Dh]).astype(bf16)
              for h in range(Hkv)]

        attn = None
        for g in range(NGRP):
            mx = [None] * G
            for j in range(NSL):
                wait(('k', g, j))
                with scope("qk"):
                    for hh in range(G):
                        s = _dot(qh[g * G + hh], k_v[g * NSL + j, hh], _NT)
                        s_s[hh, :, pl.ds(j * SROWS, SROWS)] = s
                        sm = _fold_lanes(s, jnp.maximum)
                        mx[hh] = sm if j == 0 else jnp.maximum(mx[hh], sm)
            m = [jnp.max(v, axis=-1, keepdims=True) for v in mx]
            lsum = [None] * G
            acc = [None] * G
            for j in range(NSL):
                pb = []
                with scope("exp"):
                    for hh in range(G):
                        p = jnp.exp(s_s[hh, :, pl.ds(j * SROWS, SROWS)] - m[hh])
                        ps = _fold_lanes(p, jnp.add)
                        lsum[hh] = ps if j == 0 else lsum[hh] + ps
                        pb.append(p.astype(bf16))
                    if j == NSL - 1:
                        inv = [1.0 / jnp.sum(v, axis=-1, keepdims=True) for v in lsum]
                        inv0 = [jnp.where(row == 0, v, 0.0) for v in inv]
                        inv1 = [jnp.where(row == 1, v, 0.0) for v in inv]
                if g == 0 and j == 0:
                    wait('wo')
                wait(('v', g, j))
                with scope("pv"):
                    for hh in range(G):
                        o = _dot(pb[hh], v_v[g * NSL + j, hh], _NN)
                        acc[hh] = o if j == 0 else o + acc[hh]
            with scope("wo"):
                parts = []
                for hh in range(G):
                    parts.append(acc[hh] * inv0[hh])
                    parts.append(acc[hh] * inv1[hh])
                o_cat = jnp.concatenate(parts, axis=1).astype(bf16)
                gw = G * rep * Dh
                a = _dot(o_cat, wot_v[:, pl.ds(g * gw, gw)], _NT)
                attn = a if g == 0 else a + attn

        wait(('win', 0))
        with scope("ln2"):
            attn = jnp.sum(attn, axis=0, keepdims=True)
            x1 = x + mod_s[2] * attn
            h2 = (_ln(x1) * (1.0 + mod_s[4]) + mod_s[3]).astype(bf16)
        z = None
        for i, (s0, n) in enumerate(win_groups):
            if i:
                wait(('win', i))
            with scope("win"):
                part = _dot(h2[:, s0:s0 + n], win_v[pl.ds(s0, n), :], _NN)
                z = part if z is None else part + z
        with scope("gelu"):
            z = jax.nn.gelu(z, approximate=True)
            z1 = z[:, :Fh]
            z2 = _ln(z[:, Fh:])
            gate = wsp_v[...].astype(f32) * z2 + bsp_v[...].astype(f32)
            u = (z1 * gate).astype(bf16)
        wait('gb')
        with scope("gb"):
            gb_hi = _dot(sc, gbw_v[...], _NN)
            mod_s[5] = jnp.concatenate([gb_lo, gb_hi], axis=1)
        for i, (s0, n) in enumerate(wout_groups):
            wait(('wout', i))
            with scope("wout"):
                y = _dot(u, woutt_v[pl.ds(s0, n), :], _NT)
                out = x1[:, s0:s0 + n] + mod_s[5, :, pl.ds(s0, n)] * y
                o_ref[0, :, pl.ds(s0, n)] = out[0:1, :].astype(o_ref.dtype)

      pl.run_scoped(body, pltpu.SemaphoreType.DMA((len(groups) + 4,)))

    any_spec = pl.BlockSpec(memory_space=pl.ANY)
    return pl.pallas_call(
        kernel,
        in_specs=[any_spec] * 11,
        out_specs=pl.BlockSpec(memory_space=pltpu.VMEM),
        out_shape=jax.ShapeDtypeStruct((B, Sq, D), A_x.dtype),
        scratch_shapes=[
            pltpu.VMEM((1, 1, D), bf16),
            pltpu.VMEM((1, D), bf16),
            pltpu.VMEM((1, 1), bf16),
            pltpu.VMEM((1, 1), bf16),
            pltpu.VMEM((D, MOD_EARLY), bf16),
            pltpu.VMEM((D, MOD_LATE), bf16),
            pltpu.VMEM((D, HD), bf16),
            pltpu.VMEM((NGRP * NSL, G, SROWS, Dh), bf16),
            pltpu.VMEM((NGRP * NSL, G, SROWS, Dh), bf16),
            pltpu.VMEM((D, HD), bf16),
            pltpu.VMEM((D, F), bf16),
            pltpu.VMEM((D, Fh), bf16),
            pltpu.VMEM((6, _ROWS, D), f32),
            pltpu.VMEM((G, _ROWS, W), f32),
        ],
        compiler_params=pltpu.CompilerParams(
            vmem_limit_bytes=96 * 1024 * 1024, **cfg.get('cp', {})),
    )(A_x, A_k_cache, A_v_cache, A_wq, A_wo.T, B_w_in, B_w_sp, B_b_sp.reshape(1, 1),
      B_w_out.T, c, w_mod)
  return fn


pallas_adaLN_cond__sliding_block_cached__mixer_gmlp__decode_kernel = jax.jit(make(CFG))
```

```python
import jax
import jax.numpy as jnp
from jax import lax
import jax.experimental.pallas as pl
import jax.experimental.pallas.tpu as pltpu

_NT = (((1,), (1,)), ((), ()))
_NN = (((1,), (0,)), ((), ()))
_EPS = 1e-05
_ROWS = 8
_BLK = 16

CFG = dict(
    G=4,
    sub=2,
    per=4,
    stagger=2,
    phase=0,
    align=dict(kv=14, wq=14, wo=14, win=-8, wout=-8, wmod=-8),
    mod_streams=4,
    qo_streams=4,
    win_streams=2,
    wout_streams=1,
    lag=26,
    pre=28,
    cap=60,
    win_groups=(256, 128, 64),
    wout_mxu=(128, 128),
    wout_vpu=(96, 48, 32, 16),
    vpu_reduce=(0,),
    scopes=False,
)


def _dot(a, b, dims):
    return lax.dot_general(a, b, dims, preferred_element_type=jnp.float32)


def _ln(x):
    m = jnp.mean(x, axis=-1, keepdims=True)
    d = x - m
    v = jnp.mean(d * d, axis=-1, keepdims=True)
    return d * lax.rsqrt(v + _EPS)


def _round_robin(streams):
    out = []
    for j in range(max(len(s) for s in streams)):
        for s in streams:
            if j < len(s):
                out.append(s[j])
    return out


def _split(items, n):
    m = len(items)
    return [items[i * m // n:(i + 1) * m // n] for i in range(n)]


def _ranges(sizes, r0=0):
    out = []
    for n in sizes:
        out.append((r0, n))
        r0 += n
    return out


def _tree(parts, op):
    while len(parts) > 1:
        parts = [op(parts[i], parts[i + 1]) for i in range(0, len(parts) - 1, 2)] + (
            [parts[-1]] if len(parts) % 2 else [])
    return parts[0]


def _fold_lanes(x, op):
    return _tree([x[:, i:i + 128] for i in range(0, x.shape[1], 128)], op)


def _blocks(r0, nrows, ncols, first):
    if first < 0:
        return [[(r, min(-first, r0 + nrows - r), 0, ncols)] for r in range(r0, r0 + nrows, -first)]
    nt = ncols // 128
    lo, hi = r0 // 8 * nt, (r0 + nrows) // 8 * nt
    cuts = [lo] + [t for t in range(first, hi, _BLK) if t > lo] + [hi]
    out = []
    for a, b in zip(cuts[:-1], cuts[1:]):
        rects, t = [], a
        while t < b:
            rg, ct = divmod(t, nt)
            if ct == 0 and b - t >= nt:
                k = (b - t) // nt
                rects.append((rg * 8, k * 8, 0, ncols))
                t += k * nt
            else:
                n = min(nt - ct, b - t)
                rects.append((rg * 8, 8, ct * 128, n * 128))
                t += n
        out.append(rects)
    return out


def make(cfg):
  class _Null:
    def __enter__(self): return self
    def __exit__(self, *a): return False
  def scope(name):
    return jax.named_scope(name) if cfg['scopes'] else _Null()

  def fn(
    A_x: jax.Array,
    A_k_cache: jax.Array,
    A_v_cache: jax.Array,
    A_wq: jax.Array,
    A_wo: jax.Array,
    B_x: jax.Array,
    B_w_in: jax.Array,
    B_w_sp: jax.Array,
    B_b_sp: jax.Array,
    B_w_out: jax.Array,
    c: jax.Array,
    w_mod: jax.Array,
  ):
    del B_x
    B, Sq, D = A_x.shape
    assert B == 1 and Sq == 1
    Hq, Dh = 16, 256
    Hkv, Sk = A_k_cache.shape[1], A_k_cache.shape[2]
    W = min(4096, max(256, Sk // 4))
    rep = Hq // Hkv
    assert rep == 2
    F = B_w_in.shape[-1]
    Fh = F // 2
    HD = Hq * Dh
    scale = Dh ** (-0.5)
    bf16, f32 = jnp.bfloat16, jnp.float32

    G, SUB, PER, al = cfg['G'], cfg['sub'], cfg['per'], cfg['align']
    R = _BLK * 8 * 128 // Dh
    NGRP = Hkv // G
    SROWS = SUB * PER * R
    NSL = W // SROWS
    NPS = W // (SUB * R)
    assert NSL * SROWS == W and NGRP * G == Hkv
    win_groups = _ranges(cfg['win_groups'])
    wout_mxu = _ranges(cfg['wout_mxu'])
    VP0 = sum(cfg['wout_mxu'])
    wout_vpu = _ranges(cfg['wout_vpu'], VP0)
    assert sum(cfg['win_groups']) == D and VP0 + sum(cfg['wout_vpu']) == D

    kv_shift = al['kv'] * 8 * 128 // Dh
    if kv_shift:
        kv_blocks = [[(0, kv_shift), (W - R + kv_shift, R - kv_shift)]] + [
            [(kv_shift + b * R, R)] for b in range(W // R - 1)]
    else:
        kv_blocks = [[(b * R, R)] for b in range(W // R)]

    def kernel(x_hbm, k_hbm, v_hbm, wq_hbm, wot_hbm, win_hbm, wsp_hbm, bsp_hbm,
               woutt_hbm, c_hbm, wmod_hbm,
               o_ref,
               x_v, c_v, wsp_v, bsp_v, wmod_v, wq_v, k_v, v_v, wot_v, win_v, woutt_v,
               mod_s, s_s):
      groups = {}
      need = []

      def group(name, dst):
          groups[name] = (len(groups) + 4, dst)
          return name

      def w_blocks(name, src, dst, r0, nrows, first):
          group(name, dst.at[pl.ds(r0, nrows), :])
          return [[(name, src.at[pl.ds(r, nr), pl.ds(c0, nc)], dst.at[pl.ds(r, nr), pl.ds(c0, nc)])
                   for (r, nr, c0, nc) in rects]
                  for rects in _blocks(r0, nrows, src.shape[1], first)]

      need += _round_robin(_split(
          w_blocks('wmod', wmod_hbm, wmod_v, 0, D, al['wmod']), cfg['mod_streams']))
      need += _round_robin(_round_robin([
          _split(w_blocks('wq', wq_hbm, wq_v, 0, D, al['wq']), cfg['qo_streams']),
          _split(w_blocks('wo', wot_hbm, wot_v, 0, D, al['wo']), cfg['qo_streams'])]))
      for g in range(NGRP):
          for t, hbm, vm in (('k', k_hbm, k_v), ('v', v_hbm, v_v)):
              for j in range(NSL):
                  name = group((t, g, j), vm.at[g * NSL + j])
                  for cidx in range(PER):
                      for u in range(SUB):
                          for hh in range(G):
                              pos = (j * PER + cidx + cfg['phase']
                                     + cfg['stagger'] * (u * G + hh)) % NPS
                              d0, blk = (u * PER + cidx) * R, []
                              for r, nr in kv_blocks[u * NPS + pos]:
                                  blk.append((
                                      name,
                                      hbm.at[0, g * G + hh, pl.ds(Sk - W + r, nr), :],
                                      vm.at[g * NSL + j, hh, pl.ds(d0, nr), :]))
                                  d0 += nr
                              need.append(blk)
      for i, (r0, n) in enumerate(win_groups):
          need += _round_robin(_split(
              w_blocks(('win', i), win_hbm, win_v, r0, n, al['win']), cfg['win_streams']))
      for i, (r0, n) in enumerate(wout_mxu + wout_vpu):
          need += _round_robin(_split(
              w_blocks(('wout', i), woutt_hbm, woutt_v, r0, n, al['wout']), cfg['wout_streams']))

      lag = cfg['lag']
      seq = [(e, 1 - i % 2) for i, blk in enumerate(need) for e in blk]
      seq = seq[:-lag] + [(e, 1) for e, _ in seq[-lag:]]
      lo = [e for e in seq if e[1] == 1]
      plan = lo[:lag]
      n_lo = lag
      last = {}
      for i, (e, prio) in enumerate(seq):
          last[e[0]] = i + lag - 1
          if prio == 0:
              plan.append((e, 0))
          elif n_lo < len(lo):
              plan.append(lo[n_lo])
              n_lo += 1
      assert len(plan) == len(seq)

      def body(sems):
        issued = [0]

        def issue_upto(n):
            n = min(n, len(plan))
            for (name, src, dst), prio in plan[issued[0]:n]:
                pltpu.make_async_copy(src, dst, sems.at[groups[name][0]]).start(priority=prio)
            issued[0] = max(issued[0], n)

        def wait(name):
            tag = "_".join(map(str, name)) if isinstance(name, tuple) else name
            with scope("pre_" + tag):
                issue_upto(last[name] + 2 + cfg['pre'])
            slot, dst = groups[name]
            with scope("wait_" + tag):
                pltpu.make_async_copy(dst, dst, sems.at[slot]).wait()
            with scope("post_" + tag):
                issue_upto(last[name] + 1 + cfg['cap'])

        small = [
            pltpu.make_async_copy(c_hbm, c_v, sems.at[0]),
            pltpu.make_async_copy(x_hbm, x_v, sems.at[1]),
            pltpu.make_async_copy(wsp_hbm, wsp_v, sems.at[2]),
            pltpu.make_async_copy(bsp_hbm, bsp_v, sems.at[3]),
        ]
        issue_upto(4)
        for cp in small:
            cp.start()
        issue_upto(lag + 50)
        for cp in small:
            cp.wait()
        if cfg.get('dma_only'):
            if cfg['dma_only'] == 1:
                issue_upto(len(plan))
            for name in groups:
                wait(name)
            o_ref[...] = x_v[...]
            return
        x = jnp.broadcast_to(x_v[0].astype(f32), (_ROWS, D))
        cc = jnp.broadcast_to(c_v[...].astype(f32), (_ROWS, D))
        sc = (cc * jax.nn.sigmoid(cc)).astype(bf16)
        ln_x = _ln(x)

        wait('wmod')
        mod = _dot(sc, wmod_v[...], _NN)
        for i in range(6):
            mod_s[i] = mod[:, i * D:(i + 1) * D]
        h1 = (ln_x * (1.0 + mod_s[1]) + mod_s[0]).astype(bf16)

        wait('wq')
        wait('wo')
        q = _dot(h1, wq_v[...], _NN)
        q = q.astype(bf16).astype(f32) * scale
        row = lax.broadcasted_iota(jnp.int32, (_ROWS, Dh), 0)
        qh = [jnp.where(row == 0, q[:, (2 * h) * Dh:(2 * h + 1) * Dh],
                        q[:, (2 * h + 1) * Dh:(2 * h + 2) * Dh]).astype(bf16)
              for h in range(Hkv)]

        attn = None
        for g in range(NGRP):
            mx = [None] * G
            for j in range(NSL):
                wait(('k', g, j))
                with scope("qk"):
                    for hh in range(G):
                        s = _dot(qh[g * G + hh], k_v[g * NSL + j, hh], _NT)
                        s_s[hh, :, pl.ds(j * SROWS, SROWS)] = s
                        sm = _fold_lanes(s, jnp.maximum)
                        mx[hh] = sm if j == 0 else jnp.maximum(mx[hh], sm)
            m = [jnp.max(v, axis=-1, keepdims=True) for v in mx]
            lsum = [None] * G
            acc = [None] * G
            for j in range(NSL):
                pb = []
                with scope("exp"):
                    for hh in range(G):
                        p = jnp.exp(s_s[hh, :, pl.ds(j * SROWS, SROWS)] - m[hh])
                        ps = _fold_lanes(p, jnp.add)
                        lsum[hh] = ps if j == 0 else lsum[hh] + ps
                        pb.append(p.astype(bf16))
                    if j == NSL - 1:
                        inv = [1.0 / jnp.sum(v, axis=-1, keepdims=True) for v in lsum]
                        inv0 = [jnp.where(row == 0, v, 0.0) for v in inv]
                        inv1 = [jnp.where(row == 1, v, 0.0) for v in inv]
                wait(('v', g, j))
                with scope("pv"):
                    for hh in range(G):
                        o = _dot(pb[hh], v_v[g * NSL + j, hh], _NN)
                        acc[hh] = o if j == 0 else o + acc[hh]
            if g == NGRP - 1 and cfg.get('early_win'):
                wait(('win', 0))
            with scope("wo"):
                parts = []
                for hh in range(G):
                    parts.append(acc[hh] * inv0[hh])
                    parts.append(acc[hh] * inv1[hh])
                o_cat = jnp.concatenate(parts, axis=1).astype(bf16)
                gw = G * rep * Dh
                a = _dot(o_cat, wot_v[:, pl.ds(g * gw, gw)], _NT)
                attn = a if g == 0 else a + attn

        nw = 1 if cfg.get('early_win') else 0
        wait(('win', nw))
        with scope("ln2"):
            attn = jnp.sum(attn, axis=0, keepdims=True)
            x1 = x + mod_s[2] * attn
            h2 = (_ln(x1) * (1.0 + mod_s[4]) + mod_s[3]).astype(bf16)
        z = None
        wg = list(win_groups)
        if nw:
            wg = [(0, wg[0][1] + wg[1][1])] + wg[2:]
        for i, (s0, n) in enumerate(wg):
            if i:
                wait(('win', i + nw))
            with scope("win"):
                part = _dot(h2[:, s0:s0 + n], win_v[pl.ds(s0, n), :], _NN)
                z = part if z is None else part + z
        with scope("gelu"):
            z = jax.nn.gelu(z, approximate=True)
            z1 = z[:, :Fh]
            z2 = _ln(z[:, Fh:])
            gate = wsp_v[...].astype(f32) * z2 + bsp_v[...].astype(f32)
            u = (z1 * gate).astype(bf16)

        def emit(s0, y):
            n = y.shape[1]
            out = x1[0:1, s0:s0 + n] + mod_s[5, 0:1, pl.ds(s0, n)] * y
            o_ref[0, :, pl.ds(s0, n)] = out.astype(o_ref.dtype)

        for i, (s0, n) in enumerate(wout_mxu):
            wait(('wout', i))
            with scope("wout"):
                emit(s0, _dot(u, woutt_v[pl.ds(s0, n), :], _NT)[0:1])
        uf = u.astype(f32)
        sub = lax.broadcasted_iota(jnp.int32, (_ROWS, 128), 0)
        diff = lax.broadcasted_iota(jnp.int32, (_ROWS, 128), 1) - sub

        def tile(v, t0):
            n = min(128, D - t0)
            v = v[:, t0:t0 + n]
            return v if n == 128 else jnp.concatenate(
                [v, jnp.zeros((_ROWS, 128 - n), f32)], axis=1)

        gb = mod_s[5]
        tiles = list(range(VP0 // 128 * 128, D, 128))
        oacc = {t0: jnp.where(sub == 0, tile(x1, t0), 0.0) for t0 in tiles}
        diag = {r: jnp.where(diff == r % 128, tile(gb, r // 128 * 128), 0.0)
                for r in range(VP0, D, 8)}
        pending = []
        for i, (s0, n) in enumerate(wout_vpu):
            wait(('wout', len(wout_mxu) + i))
            with scope("woutv"):
                for r in range(s0, s0 + n, 8):
                    wgt = woutt_v[pl.ds(r, 8), :].astype(f32)
                    pending.append((r, _fold_lanes(wgt * uf, jnp.add)))
                if i in cfg['vpu_reduce'] or i == len(wout_vpu) - 1:
                    for t0 in tiles:
                        terms = [jnp.sum(p, axis=-1, keepdims=True) * diag[r]
                                 for r, p in pending if t0 <= r < t0 + 128]
                        if not terms:
                            continue
                        oacc[t0] = _tree([oacc[t0]] + terms, jnp.add)
                        if s0 + n >= min(D, t0 + 128):
                            out = jnp.sum(oacc[t0], axis=0, keepdims=True)
                            lo_, hi_ = max(VP0, t0), min(D, t0 + 128)
                            o_ref[0, :, pl.ds(lo_, hi_ - lo_)] = (
                                out[:, lo_ - t0:hi_ - t0].astype(o_ref.dtype))
                    pending = []

      pl.run_scoped(body, pltpu.SemaphoreType.DMA((len(groups) + 4,)))

    any_spec = pl.BlockSpec(memory_space=pl.ANY)
    return pl.pallas_call(
        kernel,
        in_specs=[any_spec] * 11,
        out_specs=pl.BlockSpec(memory_space=pltpu.VMEM),
        out_shape=jax.ShapeDtypeStruct((B, Sq, D), A_x.dtype),
        scratch_shapes=[
            pltpu.VMEM((1, 1, D), bf16),
            pltpu.VMEM((1, D), bf16),
            pltpu.VMEM((1, 1), bf16),
            pltpu.VMEM((1, 1), bf16),
            pltpu.VMEM((D, 6 * D), bf16),
            pltpu.VMEM((D, HD), bf16),
            pltpu.VMEM((NGRP * NSL, G, SROWS, Dh), bf16),
            pltpu.VMEM((NGRP * NSL, G, SROWS, Dh), bf16),
            pltpu.VMEM((D, HD), bf16),
            pltpu.VMEM((D, F), bf16),
            pltpu.VMEM((D, Fh), bf16),
            pltpu.VMEM((6, _ROWS, D), f32),
            pltpu.VMEM((G, _ROWS, W), f32),
        ],
        compiler_params=pltpu.CompilerParams(
            vmem_limit_bytes=96 * 1024 * 1024, **cfg.get('cp', {})),
    )(A_x, A_k_cache, A_v_cache, A_wq, A_wo.T, B_w_in, B_w_sp, B_b_sp.reshape(1, 1),
      B_w_out.T, c, w_mod)
  return fn


pallas_adaLN_cond__sliding_block_cached__mixer_gmlp__decode_kernel = jax.jit(make(CFG))
```

```python
import jax
import jax.numpy as jnp
from jax import lax
import jax.experimental.pallas as pl
import jax.experimental.pallas.tpu as pltpu

_NT = (((1,), (1,)), ((), ()))
_NN = (((1,), (0,)), ((), ()))
_EPS = 1e-05
_ROWS = 8

_BLK = 16
_HEADS = 4
_SUB = 2
_PER = 4
_STAGGER = 2
_FIRST = dict(kv=14, wq=14, wo=14, wmod=1, win=-8, wout=-8)
_LAG = 26
_PRE = 28
_CAP = 60
_WIN_GROUPS = (256, 128, 64)
_WOUT_MXU = (128, 128)
_WOUT_VPU = (96, 48, 32, 16)
_VPU_REDUCE = (0, 3)


def _dot(a, b, dims):
    return lax.dot_general(a, b, dims, preferred_element_type=jnp.float32)


def _ln(x):
    m = jnp.mean(x, axis=-1, keepdims=True)
    d = x - m
    v = jnp.mean(d * d, axis=-1, keepdims=True)
    return d * lax.rsqrt(v + _EPS)


def _tree(parts, op):
    while len(parts) > 1:
        parts = [op(parts[i], parts[i + 1]) for i in range(0, len(parts) - 1, 2)] + (
            [parts[-1]] if len(parts) % 2 else [])
    return parts[0]


def _fold_lanes(x, op):
    return _tree([x[:, i:i + 128] for i in range(0, x.shape[1], 128)], op)


def _split(items, n):
    m = len(items)
    return [items[i * m // n:(i + 1) * m // n] for i in range(n)]


def _round_robin(streams):
    out = []
    for j in range(max(len(s) for s in streams)):
        out += [s[j] for s in streams if j < len(s)]
    return out


def _weave(base, extra, every):
    out = []
    for i, e in enumerate(extra):
        out += [e] + base[i * every:(i + 1) * every]
    return out + base[len(extra) * every:]


def _ranges(sizes, r0=0):
    out = []
    for n in sizes:
        out.append((r0, n))
        r0 += n
    return out


def _blocks(r0, nrows, ncols, first):
    if first < 0:
        return [[(r, min(-first, r0 + nrows - r), 0, ncols)]
                for r in range(r0, r0 + nrows, -first)]
    nt = ncols // 128
    lo, hi = r0 // 8 * nt, (r0 + nrows) // 8 * nt
    cuts = [lo] + [t for t in range(first, hi, _BLK) if t > lo] + [hi]
    out = []
    for t, end in zip(cuts[:-1], cuts[1:]):
        rects = []
        while t < end:
            rg, ct = divmod(t, nt)
            if ct == 0 and end - t >= nt:
                n = (end - t) // nt * nt
                rects.append((rg * 8, n // nt * 8, 0, ncols))
            else:
                n = min(nt - ct, end - t)
                rects.append((rg * 8, 8, ct * 128, n * 128))
            t += n
        out.append(rects)
    return out


@jax.jit
def pallas_adaLN_cond__sliding_block_cached__mixer_gmlp__decode_kernel(
    A_x: jax.Array,
    A_k_cache: jax.Array,
    A_v_cache: jax.Array,
    A_wq: jax.Array,
    A_wo: jax.Array,
    B_x: jax.Array,
    B_w_in: jax.Array,
    B_w_sp: jax.Array,
    B_b_sp: jax.Array,
    B_w_out: jax.Array,
    c: jax.Array,
    w_mod: jax.Array,
):
    del B_x
    B, Sq, D = A_x.shape
    Hq, Dh = 16, 256
    Hkv, Sk = A_k_cache.shape[1], A_k_cache.shape[2]
    W = min(4096, max(256, Sk // 4))
    rep = Hq // Hkv
    F = B_w_in.shape[-1]
    Fh = F // 2
    HD = Hq * Dh
    scale = Dh ** (-0.5)
    bf16, f32 = jnp.bfloat16, jnp.float32
    assert B == 1 and Sq == 1 and rep == 2

    G = _HEADS
    R = _BLK * 8 * 128 // Dh
    n_grp = Hkv // G
    s_rows = _SUB * _PER * R
    n_sl = W // s_rows
    n_ps = W // (_SUB * R)
    win_groups = _ranges(_WIN_GROUPS)
    wout_mxu = _ranges(_WOUT_MXU)
    vp0 = sum(_WOUT_MXU)
    wout_vpu = _ranges(_WOUT_VPU, vp0)
    assert n_sl * s_rows == W and n_grp * G == Hkv
    assert sum(_WIN_GROUPS) == D and vp0 + sum(_WOUT_VPU) == D

    sh = _FIRST['kv'] * 8 * 128 // Dh
    kv_blocks = [[(0, sh), (W - R + sh, R - sh)]] + [
        [(sh + b * R, R)] for b in range(W // R - 1)]

    def kernel(x_hbm, k_hbm, v_hbm, wq_hbm, wot_hbm, win_hbm, wsp_hbm, bsp_hbm,
               woutt_hbm, c_hbm, wmod_hbm,
               o_ref,
               x_v, c_v, wsp_v, bsp_v, wmod_v, wq_v, k_v, v_v, wot_v, win_v, woutt_v,
               mod_s, s_s):
        n_small = 4
        groups = {}
        need = []

        def group(name, dst):
            groups[name] = (n_small + len(groups), dst)

        def w_blocks(name, src, dst, r0, nrows, first):
            group(name, dst.at[pl.ds(r0, nrows), :])
            return [[(name, src.at[pl.ds(r, nr), pl.ds(c0, nc)],
                      dst.at[pl.ds(r, nr), pl.ds(c0, nc)]) for r, nr, c0, nc in rects]
                    for rects in _blocks(r0, nrows, src.shape[1], first)]

        need += _weave(
            _round_robin(_round_robin([
                _split(w_blocks('wq', wq_hbm, wq_v, 0, D, _FIRST['wq']), 4),
                _split(w_blocks('wo', wot_hbm, wot_v, 0, D, _FIRST['wo']), 4)])),
            _round_robin(_split(w_blocks('wmod', wmod_hbm, wmod_v, 0, D, _FIRST['wmod']), 3)),
            2)
        for g in range(n_grp):
            for t, hbm, vm in (('k', k_hbm, k_v), ('v', v_hbm, v_v)):
                for j in range(n_sl):
                    group((t, g, j), vm.at[g * n_sl + j])
                    for i in range(_PER):
                        for u in range(_SUB):
                            for hh in range(G):
                                pos = (j * _PER + i + _STAGGER * (u * G + hh)) % n_ps
                                d0, blk = (u * _PER + i) * R, []
                                for r, nr in kv_blocks[u * n_ps + pos]:
                                    blk.append((
                                        (t, g, j),
                                        hbm.at[0, g * G + hh, pl.ds(Sk - W + r, nr), :],
                                        vm.at[g * n_sl + j, hh, pl.ds(d0, nr), :]))
                                    d0 += nr
                                need.append(blk)
        for i, (r0, n) in enumerate(win_groups):
            need += _round_robin(_split(
                w_blocks(('win', i), win_hbm, win_v, r0, n, _FIRST['win']), 2))
        for i, (r0, n) in enumerate(wout_mxu + wout_vpu):
            need += w_blocks(('wout', i), woutt_hbm, woutt_v, r0, n, _FIRST['wout'])

        seq = [(e, 1 - i % 2) for i, blk in enumerate(need) for e in blk]
        seq = seq[:-_LAG] + [(e, 1) for e, _ in seq[-_LAG:]]
        low = [e for e in seq if e[1] == 1]
        plan, n_low = low[:_LAG], _LAG
        done_at = {}
        for i, (e, prio) in enumerate(seq):
            done_at[e[0]] = i + _LAG
            if prio == 0:
                plan.append((e, 0))
            elif n_low < len(low):
                plan.append(low[n_low])
                n_low += 1
        assert len(plan) == len(seq)
        assert all(i <= done_at[e[0]] for i, (e, _) in enumerate(plan))

        def body(sems):
            issued = [0]

            def issue_upto(n):
                n = min(n, len(plan))
                for (name, src, dst), prio in plan[issued[0]:n]:
                    pltpu.make_async_copy(
                        src, dst, sems.at[groups[name][0]]).start(priority=prio)
                issued[0] = max(issued[0], n)

            def wait(name):
                slot, dst = groups[name]
                issue_upto(done_at[name] + 1 + _PRE)
                pltpu.make_async_copy(dst, dst, sems.at[slot]).wait()
                issue_upto(done_at[name] + _CAP)

            small = [
                pltpu.make_async_copy(src, dst, sems.at[i]) for i, (src, dst) in enumerate((
                    (c_hbm, c_v), (x_hbm, x_v), (wsp_hbm, wsp_v), (bsp_hbm, bsp_v)))]
            issue_upto(4)
            for cp in small:
                cp.start()
            issue_upto(_LAG + 50)
            for cp in small:
                cp.wait()

            x = jnp.broadcast_to(x_v[0].astype(f32), (_ROWS, D))
            cc = jnp.broadcast_to(c_v[...].astype(f32), (_ROWS, D))
            sc = (cc * jax.nn.sigmoid(cc)).astype(bf16)
            ln_x = _ln(x)

            wait('wmod')
            mod = _dot(sc, wmod_v[...], _NN)
            for i in range(6):
                mod_s[i] = mod[:, i * D:(i + 1) * D]
            h1 = (ln_x * (1.0 + mod_s[1]) + mod_s[0]).astype(bf16)

            wait('wq')
            wait('wo')
            q = _dot(h1, wq_v[...], _NN).astype(bf16).astype(f32) * scale
            row = lax.broadcasted_iota(jnp.int32, (_ROWS, Dh), 0)
            qh = [jnp.where(row == 0, q[:, (2 * h) * Dh:(2 * h + 1) * Dh],
                            q[:, (2 * h + 1) * Dh:(2 * h + 2) * Dh]).astype(bf16)
                  for h in range(Hkv)]

            attn = None
            for g in range(n_grp):
                mx = [None] * G
                for j in range(n_sl):
                    wait(('k', g, j))
                    for hh in range(G):
                        s = _dot(qh[g * G + hh], k_v[g * n_sl + j, hh], _NT)
                        s_s[hh, :, pl.ds(j * s_rows, s_rows)] = s
                        sm = _fold_lanes(s, jnp.maximum)
                        mx[hh] = sm if j == 0 else jnp.maximum(mx[hh], sm)
                m = [jnp.max(v, axis=-1, keepdims=True) for v in mx]
                lsum, acc = [None] * G, [None] * G
                for j in range(n_sl):
                    pb = []
                    for hh in range(G):
                        p = jnp.exp(s_s[hh, :, pl.ds(j * s_rows, s_rows)] - m[hh])
                        ps = _fold_lanes(p, jnp.add)
                        lsum[hh] = ps if j == 0 else lsum[hh] + ps
                        pb.append(p.astype(bf16))
                    if j == n_sl - 1:
                        inv = [1.0 / jnp.sum(v, axis=-1, keepdims=True) for v in lsum]
                        inv0 = [jnp.where(row == 0, v, 0.0) for v in inv]
                        inv1 = [jnp.where(row == 1, v, 0.0) for v in inv]
                    wait(('v', g, j))
                    for hh in range(G):
                        o = _dot(pb[hh], v_v[g * n_sl + j, hh], _NN)
                        acc[hh] = o if j == 0 else o + acc[hh]
                o_cat = jnp.concatenate(
                    [acc[hh] * iv[hh] for hh in range(G) for iv in (inv0, inv1)],
                    axis=1).astype(bf16)
                gw = G * rep * Dh
                a = _dot(o_cat, wot_v[:, pl.ds(g * gw, gw)], _NT)
                attn = a if g == 0 else a + attn

            wait(('win', 0))
            x1 = x + mod_s[2] * jnp.sum(attn, axis=0, keepdims=True)
            h2 = (_ln(x1) * (1.0 + mod_s[4]) + mod_s[3]).astype(bf16)
            z = None
            for i, (s0, n) in enumerate(win_groups):
                if i:
                    wait(('win', i))
                part = _dot(h2[:, s0:s0 + n], win_v[pl.ds(s0, n), :], _NN)
                z = part if z is None else part + z
            z = jax.nn.gelu(z, approximate=True)
            gate = wsp_v[...].astype(f32) * _ln(z[:, Fh:]) + bsp_v[...].astype(f32)
            u = (z[:, :Fh] * gate).astype(bf16)

            for i, (s0, n) in enumerate(wout_mxu):
                wait(('wout', i))
                y = _dot(u, woutt_v[pl.ds(s0, n), :], _NT)[0:1]
                out = x1[0:1, s0:s0 + n] + mod_s[5, 0:1, pl.ds(s0, n)] * y
                o_ref[0, :, pl.ds(s0, n)] = out.astype(o_ref.dtype)

            uf = u.astype(f32)
            sub = lax.broadcasted_iota(jnp.int32, (_ROWS, 128), 0)
            diff = lax.broadcasted_iota(jnp.int32, (_ROWS, 128), 1) - sub

            def tile(v, t0):
                n = min(128, D - t0)
                v = v[:, t0:t0 + n]
                return v if n == 128 else jnp.concatenate(
                    [v, jnp.zeros((_ROWS, 128 - n), f32)], axis=1)

            gb = mod_s[5]
            tiles = list(range(vp0 // 128 * 128, D, 128))
            oacc = {t0: jnp.where(sub == 0, tile(x1, t0), 0.0) for t0 in tiles}
            diag = {r: jnp.where(diff == r % 128, tile(gb, r // 128 * 128), 0.0)
                    for r in range(vp0, D, 8)}
            pending = []
            for i, (s0, n) in enumerate(wout_vpu):
                wait(('wout', len(wout_mxu) + i))
                for r in range(s0, s0 + n, 8):
                    wgt = woutt_v[pl.ds(r, 8), :].astype(f32)
                    pending.append((r, _fold_lanes(wgt * uf, jnp.add)))
                if i not in _VPU_REDUCE:
                    continue
                for t0 in tiles:
                    terms = [jnp.sum(p, axis=-1, keepdims=True) * diag[r]
                             for r, p in pending if t0 <= r < t0 + 128]
                    if not terms:
                        continue
                    oacc[t0] = _tree([oacc[t0]] + terms, jnp.add)
                    lo, hi = max(vp0, t0), min(D, t0 + 128)
                    if s0 + n >= hi:
                        out = jnp.sum(oacc[t0], axis=0, keepdims=True)
                        o_ref[0, :, pl.ds(lo, hi - lo)] = (
                            out[:, lo - t0:hi - t0].astype(o_ref.dtype))
                pending = []
            assert not pending and issued[0] == len(plan)

        pl.run_scoped(body, pltpu.SemaphoreType.DMA((n_small + len(groups),)))

    return pl.pallas_call(
        kernel,
        in_specs=[pl.BlockSpec(memory_space=pl.ANY)] * 11,
        out_specs=pl.BlockSpec(memory_space=pltpu.VMEM),
        out_shape=jax.ShapeDtypeStruct((B, Sq, D), A_x.dtype),
        scratch_shapes=[
            pltpu.VMEM((1, 1, D), bf16),
            pltpu.VMEM((1, D), bf16),
            pltpu.VMEM((1, 1), bf16),
            pltpu.VMEM((1, 1), bf16),
            pltpu.VMEM((D, 6 * D), bf16),
            pltpu.VMEM((D, HD), bf16),
            pltpu.VMEM((n_grp * n_sl, G, s_rows, Dh), bf16),
            pltpu.VMEM((n_grp * n_sl, G, s_rows, Dh), bf16),
            pltpu.VMEM((D, HD), bf16),
            pltpu.VMEM((D, F), bf16),
            pltpu.VMEM((D, Fh), bf16),
            pltpu.VMEM((6, _ROWS, D), f32),
            pltpu.VMEM((G, _ROWS, W), f32),
        ],
        compiler_params=pltpu.CompilerParams(vmem_limit_bytes=64 * 1024 * 1024),
    )(A_x, A_k_cache, A_v_cache, A_wq, A_wo.T, B_w_in, B_w_sp, B_b_sp.reshape(1, 1),
      B_w_out.T, c, w_mod)
```

```python
import jax
import jax.numpy as jnp
from jax import lax
import jax.experimental.pallas as pl
import jax.experimental.pallas.tpu as pltpu

_NT = (((1,), (1,)), ((), ()))
_NN = (((1,), (0,)), ((), ()))
_EPS = 1e-05
_ROWS = 8

_BLK = 16
_HEADS = 4
_SUB = 2
_PER = 4
_STAGGER = -2
_FIRST = dict(kv=14, wq=14, wo=14, wmod=1, wout=-8)
_LAG = 26
_PRE = 28
_CAP = 60
_WIN_SHARES = ((88, 88, 80), (40, 40, 48), (24, 24, 16))
_WOUT_MXU = (128, 128)
_WOUT_VPU = (96, 48, 32, 16)
_VPU_REDUCE = (0, 3)


def _dot(a, b, dims):
    return lax.dot_general(a, b, dims, preferred_element_type=jnp.float32)


def _ln(x):
    m = jnp.mean(x, axis=-1, keepdims=True)
    d = x - m
    v = jnp.mean(d * d, axis=-1, keepdims=True)
    return d * lax.rsqrt(v + _EPS)


def _tree(parts, op):
    while len(parts) > 1:
        parts = [op(parts[i], parts[i + 1]) for i in range(0, len(parts) - 1, 2)] + (
            [parts[-1]] if len(parts) % 2 else [])
    return parts[0]


def _fold_lanes(x, op):
    return _tree([x[:, i:i + 128] for i in range(0, x.shape[1], 128)], op)


def _split(items, n):
    m = len(items)
    return [items[i * m // n:(i + 1) * m // n] for i in range(n)]


def _round_robin(streams):
    out = []
    for j in range(max(len(s) for s in streams)):
        out += [s[j] for s in streams if j < len(s)]
    return out


def _weave(base, extra, every):
    out = []
    for i, e in enumerate(extra):
        out += [e] + base[i * every:(i + 1) * every]
    return out + base[len(extra) * every:]


def _ranges(sizes, r0=0):
    out = []
    for n in sizes:
        out.append((r0, n))
        r0 += n
    return out


def _blocks(r0, nrows, ncols, first):
    if first < 0:
        return [[(r, min(-first, r0 + nrows - r), 0, ncols)]
                for r in range(r0, r0 + nrows, -first)]
    nt = ncols // 128
    lo, hi = r0 // 8 * nt, (r0 + nrows) // 8 * nt
    cuts = [lo] + [t for t in range(first, hi, _BLK) if t > lo] + [hi]
    out = []
    for t, end in zip(cuts[:-1], cuts[1:]):
        rects = []
        while t < end:
            rg, ct = divmod(t, nt)
            if ct == 0 and end - t >= nt:
                n = (end - t) // nt * nt
                rects.append((rg * 8, n // nt * 8, 0, ncols))
            else:
                n = min(nt - ct, end - t)
                rects.append((rg * 8, 8, ct * 128, n * 128))
            t += n
        out.append(rects)
    return out


@jax.jit
def pallas_adaLN_cond__sliding_block_cached__mixer_gmlp__decode_kernel(
    A_x: jax.Array,
    A_k_cache: jax.Array,
    A_v_cache: jax.Array,
    A_wq: jax.Array,
    A_wo: jax.Array,
    B_x: jax.Array,
    B_w_in: jax.Array,
    B_w_sp: jax.Array,
    B_b_sp: jax.Array,
    B_w_out: jax.Array,
    c: jax.Array,
    w_mod: jax.Array,
):
    del B_x
    B, Sq, D = A_x.shape
    Hq, Dh = 16, 256
    Hkv, Sk = A_k_cache.shape[1], A_k_cache.shape[2]
    W = min(4096, max(256, Sk // 4))
    rep = Hq // Hkv
    F = B_w_in.shape[-1]
    Fh = F // 2
    HD = Hq * Dh
    scale = Dh ** (-0.5)
    bf16, f32 = jnp.bfloat16, jnp.float32
    assert B == 1 and Sq == 1 and rep == 2

    G = _HEADS
    R = _BLK * 8 * 128 // Dh
    n_grp = Hkv // G
    s_rows = _SUB * _PER * R
    n_sl = W // s_rows
    n_ps = W // (_SUB * R)
    wout_mxu = _ranges(_WOUT_MXU)
    vp0 = sum(_WOUT_MXU)
    wout_vpu = _ranges(_WOUT_VPU, vp0)
    assert n_sl * s_rows == W and n_grp * G == Hkv
    assert vp0 + sum(_WOUT_VPU) == D

    win_groups = _ranges([sum(sh) for sh in _WIN_SHARES])
    src0 = [r0 for r0, _ in _ranges([sum(col) for col in zip(*_WIN_SHARES)])]
    win_parts = []
    for (dst0, _), shares in zip(win_groups, _WIN_SHARES):
        win_parts.append([(a, b, n) for a, (b, n) in zip(src0, _ranges(shares, dst0))])
        src0 = [a + n for a, n in zip(src0, shares)]
    assert src0[-1] == D

    sh = _FIRST['kv'] * 8 * 128 // Dh
    kv_blocks = [[(0, sh), (W - R + sh, R - sh)]] + [
        [(sh + b * R, R)] for b in range(W // R - 1)]

    def kernel(x_hbm, k_hbm, v_hbm, wq_hbm, wot_hbm, win_hbm, wsp_hbm, bsp_hbm,
               woutt_hbm, c_hbm, wmod_hbm,
               o_ref,
               x_v, c_v, wsp_v, bsp_v, wmod_v, wq_v, k_v, v_v, wot_v, win_v, woutt_v,
               mod_s, s_s):
        n_small = 4
        groups = {}
        need = []

        def group(name, dst):
            groups[name] = (n_small + len(groups), dst)

        def w_blocks(name, src, dst, r0, nrows, first):
            group(name, dst.at[pl.ds(r0, nrows), :])
            return [[(name, src.at[pl.ds(r, nr), pl.ds(c0, nc)],
                      dst.at[pl.ds(r, nr), pl.ds(c0, nc)]) for r, nr, c0, nc in rects]
                    for rects in _blocks(r0, nrows, src.shape[1], first)]

        need += _weave(
            _round_robin(_round_robin([
                _split(w_blocks('wq', wq_hbm, wq_v, 0, D, _FIRST['wq']), 4),
                _split(w_blocks('wo', wot_hbm, wot_v, 0, D, _FIRST['wo']), 4)])),
            _round_robin(_split(w_blocks('wmod', wmod_hbm, wmod_v, 0, D, _FIRST['wmod']), 3)),
            2)
        for g in range(n_grp):
            for t, hbm, vm in (('k', k_hbm, k_v), ('v', v_hbm, v_v)):
                for j in range(n_sl):
                    group((t, g, j), vm.at[g * n_sl + j])
                    for i in range(_PER):
                        for u in range(_SUB):
                            for hh in range(G):
                                pos = (j * _PER + i + _STAGGER * (u * G + hh)) % n_ps
                                d0, blk = (u * _PER + i) * R, []
                                for r, nr in kv_blocks[u * n_ps + pos]:
                                    blk.append((
                                        (t, g, j),
                                        hbm.at[0, g * G + hh, pl.ds(Sk - W + r, nr), :],
                                        vm.at[g * n_sl + j, hh, pl.ds(d0, nr), :]))
                                    d0 += nr
                                need.append(blk)
        for i, (r0, n) in enumerate(win_groups):
            group(('win', i), win_v.at[pl.ds(r0, n), :])
            need += _round_robin([
                [[(('win', i), win_hbm.at[pl.ds(a + r, 8), :], win_v.at[pl.ds(b + r, 8), :])]
                 for r in range(0, nr, 8)] for a, b, nr in win_parts[i]])
        for i, (r0, n) in enumerate(wout_mxu + wout_vpu):
            need += w_blocks(('wout', i), woutt_hbm, woutt_v, r0, n, _FIRST['wout'])

        seq = [(e, 1 - i % 2) for i, blk in enumerate(need) for e in blk]
        seq = seq[:-_LAG] + [(e, 1) for e, _ in seq[-_LAG:]]
        low = [e for e in seq if e[1] == 1]
        plan, n_low = low[:_LAG], _LAG
        done_at = {}
        for i, (e, prio) in enumerate(seq):
            done_at[e[0]] = i + _LAG
            if prio == 0:
                plan.append((e, 0))
            elif n_low < len(low):
                plan.append(low[n_low])
                n_low += 1
        assert len(plan) == len(seq)
        assert all(i <= done_at[e[0]] for i, (e, _) in enumerate(plan))

        def body(sems):
            issued = [0]

            def issue_upto(n):
                n = min(n, len(plan))
                for (name, src, dst), prio in plan[issued[0]:n]:
                    pltpu.make_async_copy(
                        src, dst, sems.at[groups[name][0]]).start(priority=prio)
                issued[0] = max(issued[0], n)

            def wait(name):
                slot, dst = groups[name]
                issue_upto(done_at[name] + 1 + _PRE)
                pltpu.make_async_copy(dst, dst, sems.at[slot]).wait()
                issue_upto(done_at[name] + _CAP)

            small = [
                pltpu.make_async_copy(src, dst, sems.at[i]) for i, (src, dst) in enumerate((
                    (c_hbm, c_v), (x_hbm, x_v), (wsp_hbm, wsp_v), (bsp_hbm, bsp_v)))]
            issue_upto(4)
            for cp in small:
                cp.start()
            issue_upto(_LAG + 50)
            for cp in small:
                cp.wait()

            x = jnp.broadcast_to(x_v[0].astype(f32), (_ROWS, D))
            cc = jnp.broadcast_to(c_v[...].astype(f32), (_ROWS, D))
            sc = (cc * jax.nn.sigmoid(cc)).astype(bf16)
            ln_x = _ln(x)

            wait('wmod')
            mod = _dot(sc, wmod_v[...], _NN)
            for i in range(6):
                mod_s[i] = mod[:, i * D:(i + 1) * D]
            h1 = (ln_x * (1.0 + mod_s[1]) + mod_s[0]).astype(bf16)

            wait('wq')
            wait('wo')
            q = _dot(h1, wq_v[...], _NN).astype(bf16).astype(f32) * scale
            row = lax.broadcasted_iota(jnp.int32, (_ROWS, Dh), 0)
            qh = [jnp.where(row == 0, q[:, (2 * h) * Dh:(2 * h + 1) * Dh],
                            q[:, (2 * h + 1) * Dh:(2 * h + 2) * Dh]).astype(bf16)
                  for h in range(Hkv)]

            attn = None
            for g in range(n_grp):
                mx = [None] * G
                for j in range(n_sl):
                    wait(('k', g, j))
                    for hh in range(G):
                        s = _dot(qh[g * G + hh], k_v[g * n_sl + j, hh], _NT)
                        s_s[hh, :, pl.ds(j * s_rows, s_rows)] = s
                        sm = _fold_lanes(s, jnp.maximum)
                        mx[hh] = sm if j == 0 else jnp.maximum(mx[hh], sm)
                m = [jnp.max(v, axis=-1, keepdims=True) for v in mx]
                lsum, acc = [None] * G, [None] * G
                for j in range(n_sl):
                    pb = []
                    for hh in range(G):
                        p = jnp.exp(s_s[hh, :, pl.ds(j * s_rows, s_rows)] - m[hh])
                        ps = _fold_lanes(p, jnp.add)
                        lsum[hh] = ps if j == 0 else lsum[hh] + ps
                        pb.append(p.astype(bf16))
                    if j == n_sl - 1:
                        inv = [1.0 / jnp.sum(v, axis=-1, keepdims=True) for v in lsum]
                        inv0 = [jnp.where(row == 0, v, 0.0) for v in inv]
                        inv1 = [jnp.where(row == 1, v, 0.0) for v in inv]
                    wait(('v', g, j))
                    for hh in range(G):
                        o = _dot(pb[hh], v_v[g * n_sl + j, hh], _NN)
                        acc[hh] = o if j == 0 else o + acc[hh]
                o_cat = jnp.concatenate(
                    [acc[hh] * iv[hh] for hh in range(G) for iv in (inv0, inv1)],
                    axis=1).astype(bf16)
                gw = G * rep * Dh
                a = _dot(o_cat, wot_v[:, pl.ds(g * gw, gw)], _NT)
                attn = a if g == 0 else a + attn

            x1 = x + mod_s[2] * jnp.sum(attn, axis=0, keepdims=True)
            h2 = _ln(x1) * (1.0 + mod_s[4]) + mod_s[3]
            h2 = jnp.concatenate(
                [h2[:, a:a + nr] for parts in win_parts for a, _, nr in parts],
                axis=1).astype(bf16)
            z = None
            for i, (s0, n) in enumerate(win_groups):
                wait(('win', i))
                part = _dot(h2[:, s0:s0 + n], win_v[pl.ds(s0, n), :], _NN)
                z = part if z is None else part + z
            z = jax.nn.gelu(z, approximate=True)
            gate = wsp_v[...].astype(f32) * _ln(z[:, Fh:]) + bsp_v[...].astype(f32)
            u = (z[:, :Fh] * gate).astype(bf16)

            for i, (s0, n) in enumerate(wout_mxu):
                wait(('wout', i))
                y = _dot(u, woutt_v[pl.ds(s0, n), :], _NT)[0:1]
                out = x1[0:1, s0:s0 + n] + mod_s[5, 0:1, pl.ds(s0, n)] * y
                o_ref[0, :, pl.ds(s0, n)] = out.astype(o_ref.dtype)

            uf = u.astype(f32)
            sub = lax.broadcasted_iota(jnp.int32, (_ROWS, 128), 0)
            diff = lax.broadcasted_iota(jnp.int32, (_ROWS, 128), 1) - sub

            def tile(v, t0):
                n = min(128, D - t0)
                v = v[:, t0:t0 + n]
                return v if n == 128 else jnp.concatenate(
                    [v, jnp.zeros((_ROWS, 128 - n), f32)], axis=1)

            gb = mod_s[5]
            tiles = list(range(vp0 // 128 * 128, D, 128))
            oacc = {t0: jnp.where(sub == 0, tile(x1, t0), 0.0) for t0 in tiles}
            diag = {r: jnp.where(diff == r % 128, tile(gb, r // 128 * 128), 0.0)
                    for r in range(vp0, D, 8)}
            pending = []
            for i, (s0, n) in enumerate(wout_vpu):
                wait(('wout', len(wout_mxu) + i))
                for r in range(s0, s0 + n, 8):
                    wgt = woutt_v[pl.ds(r, 8), :].astype(f32)
                    pending.append((r, _fold_lanes(wgt * uf, jnp.add)))
                if i not in _VPU_REDUCE:
                    continue
                for t0 in tiles:
                    terms = [jnp.sum(p, axis=-1, keepdims=True) * diag[r]
                             for r, p in pending if t0 <= r < t0 + 128]
                    if not terms:
                        continue
                    oacc[t0] = _tree([oacc[t0]] + terms, jnp.add)
                    lo, hi = max(vp0, t0), min(D, t0 + 128)
                    if s0 + n >= hi:
                        out = jnp.sum(oacc[t0], axis=0, keepdims=True)
                        o_ref[0, :, pl.ds(lo, hi - lo)] = (
                            out[:, lo - t0:hi - t0].astype(o_ref.dtype))
                pending = []
            assert not pending and issued[0] == len(plan)

        pl.run_scoped(body, pltpu.SemaphoreType.DMA((n_small + len(groups),)))

    return pl.pallas_call(
        kernel,
        in_specs=[pl.BlockSpec(memory_space=pl.ANY)] * 11,
        out_specs=pl.BlockSpec(memory_space=pltpu.VMEM),
        out_shape=jax.ShapeDtypeStruct((B, Sq, D), A_x.dtype),
        scratch_shapes=[
            pltpu.VMEM((1, 1, D), bf16),
            pltpu.VMEM((1, D), bf16),
            pltpu.VMEM((1, 1), bf16),
            pltpu.VMEM((1, 1), bf16),
            pltpu.VMEM((D, 6 * D), bf16),
            pltpu.VMEM((D, HD), bf16),
            pltpu.VMEM((n_grp * n_sl, G, s_rows, Dh), bf16),
            pltpu.VMEM((n_grp * n_sl, G, s_rows, Dh), bf16),
            pltpu.VMEM((D, HD), bf16),
            pltpu.VMEM((D, F), bf16),
            pltpu.VMEM((D, Fh), bf16),
            pltpu.VMEM((6, _ROWS, D), f32),
            pltpu.VMEM((G, _ROWS, W), f32),
        ],
        compiler_params=pltpu.CompilerParams(vmem_limit_bytes=64 * 1024 * 1024),
    )(A_x, A_k_cache, A_v_cache, A_wq, A_wo.T, B_w_in, B_w_sp, B_b_sp.reshape(1, 1),
      B_w_out.T, c, w_mod)
```
